```python
import os as _os
_os.environ.setdefault("JAX_PLATFORMS", "cpu")
import jax
import jax.numpy as jnp

def _softmax(x, axis=-1):
    return jax.nn.softmax(x, axis=axis)
def _gelu(x):
    return jax.nn.gelu(x, approximate=True)
def _silu(x):
    return jax.nn.silu(x)
def _sigmoid(x):
    return jax.nn.sigmoid(x)
def _layernorm(x, axis=-1, eps=1e-5):
    m = jnp.mean(x, axis=axis, keepdims=True)
    v = jnp.var(x, axis=axis, keepdims=True)
    return (x - m) / jnp.sqrt(v + eps)
def _scatter_add(tgt, idx, src, axis=0):
    return tgt.at[idx].add(src)
def _segment_sum(src, seg, n):
    return jax.ops.segment_sum(src, seg, n)
class _Rng:
    def __init__(self, key):
        self._k = key
    def _next(self):
        self._k, sub = jax.random.split(self._k)
        return sub
    def normal(self, shape):
        return jax.random.normal(self._next(), shape, dtype=jnp.bfloat16)
    def randint(self, lo, hi, shape):
        return jax.random.randint(self._next(), shape, lo, hi, dtype=jnp.int32)
    def uniform(self, shape, lo=0.0, hi=1.0):
        return jax.random.uniform(self._next(), shape, jnp.bfloat16, lo, hi)
    def permutation(self, n):
        return jax.random.permutation(self._next(), n)


kernel_name = 'sequential_preLN__spectral_gfnet__glu_gated_bilinear__prompt'

def setup_inputs():
    _rng = _Rng(jax.random.key(int.from_bytes(__import__("os").urandom(4), "little")))
    _w = (lambda a: (lambda t: t.astype(jnp.bfloat16) if jnp.issubdtype(t.dtype, jnp.floating) else t)(jnp.asarray(a)))
    def _A_setup():
        B, S, D = 1, 2048, 448
        Df = D // 2 + 1
        return {
            "x": _w((lambda *s: _rng.normal(s) * 0.05)(B, S, D)),
            "w_r": _w((lambda *s: _rng.normal(s) * 0.2)(S, Df) * 0.02),
            "w_i": _w((lambda *s: _rng.normal(s) * 0.2)(S, Df) * 0.02),
        }
    _A_in = _A_setup()

    def _B_setup():
        B, S, D, F = 1, 2048, 448, 1792
        return {
            "x": _w((lambda *s: _rng.normal(s) * 0.05)(B, S, D)),
            "w_gate": _w((lambda *s: _rng.normal(s) * 0.05)(D, F) * (D ** -0.5)),
            "w_up": _w((lambda *s: _rng.normal(s) * 0.05)(D, F) * (D ** -0.5)),
            "w_down": _w((lambda *s: _rng.normal(s) * 0.05)(F, D) * (F ** -0.5)),
        }
    _B_in = _B_setup()

    return {
        "A_x": _A_in["x"],
        "A_w_r": _A_in["w_r"],
        "A_w_i": _A_in["w_i"],
        "B_x": _B_in["x"],
        "B_w_gate": _B_in["w_gate"],
        "B_w_up": _B_in["w_up"],
        "B_w_down": _B_in["w_down"],
    }

def reference(A_x, A_w_r, A_w_i, B_x, B_w_gate, B_w_up, B_w_down):
    def _A_ref(x, w_r, w_i):
        B, S, D = x.shape
        X = (lambda x, axes=(-2,-1): jnp.fft.rfft2(x.astype(jnp.float32), axes=axes))(x, axes=(-2, -1))
        W = w_r + 1j * w_i
        X = X * W
        y = (lambda x, s, axes=(-2,-1): jnp.fft.irfft2(x, s=s, axes=axes).astype(jnp.bfloat16))(X, (S, D), axes=(-2, -1))
        return y

    def _B_ref(x, w_gate, w_up, w_down):
        g = jnp.einsum("bsd,df->bsf", x, w_gate)
        u = jnp.einsum("bsd,df->bsf", x, w_up)
        h = g * u
        return jnp.einsum("bsf,fd->bsd", h, w_down)

    x = A_x
    h = x + _A_ref(_layernorm(x, axis=-1), A_w_r, A_w_i)
    h2 = h + _B_ref(_layernorm(h, axis=-1), B_w_gate, B_w_up, B_w_down)
    return h2
```

```python
import functools

import numpy as np
import jax
import jax.numpy as jnp
import jax.experimental.pallas as pl
import jax.experimental.pallas.tpu as pltpu

S = 2048
D = 448
DF = D // 2 + 1
CP = 256
FF = 1792
N1 = 128
N2 = 16
NG = S // N1
TM = 512
TA = 512
EPS = 1e-5


@functools.lru_cache(maxsize=1)
def _consts():
    ang = 2.0 * np.pi * np.outer(np.arange(D), np.arange(DF)) / D
    cd = np.zeros((D, 2 * CP), np.float64)
    cd[:, :DF] = np.cos(ang)
    cd[:, CP:CP + DF] = -np.sin(ang)
    ck = np.full((DF,), 2.0)
    ck[0] = 1.0
    ck[DF - 1] = 1.0
    idm = np.zeros((2 * CP, D), np.float64)
    idm[:DF, :] = (ck[:, None] * np.cos(ang.T)) / (S * D)
    sin_part = -(ck[:, None] * np.sin(ang.T)) / (S * D)
    sin_part[0, :] = 0.0
    sin_part[DF - 1, :] = 0.0
    idm[CP:CP + DF, :] = sin_part
    idt = idm.T.copy()
    a = 2.0 * np.pi * np.outer(np.arange(N1), np.arange(N1)) / N1
    f1 = np.concatenate([np.cos(a), -np.sin(a)], axis=0)
    f1i = np.concatenate([np.cos(a), np.sin(a)], axis=0)
    gs = np.zeros((NG, 2 * N1, N1), np.float64)
    hs = np.zeros((NG, 2 * N1, N1), np.float64)
    n2 = np.arange(N2)
    for g in range(NG):
        m = np.zeros((N1, N1), np.complex128)
        for j in range(8):
            k1 = 8 * g + j
            for k2 in range(N2):
                m[8 * k2 + j, 16 * j + n2] = np.exp(
                    -2j * np.pi * (n2 * k2 / N2 + n2 * k1 / S))
        gs[g, :N1] = m.real
        gs[g, N1:] = m.imag
        h = m.conj().T
        hs[g, :N1] = h.real
        hs[g, N1:] = h.imag
    bf = lambda t: np.asarray(t, dtype=jnp.bfloat16)
    return bf(cd), bf(idt), bf(f1), bf(f1i), bf(gs), bf(hs)


def _ln_t(xf):
    m = jnp.mean(xf, axis=0, keepdims=True)
    xc = xf - m
    v = jnp.mean(xc * xc, axis=0, keepdims=True)
    return xc * jax.lax.rsqrt(v + EPS)


def _cmul_split(p):
    re = p[:N1, :CP] - p[N1:, CP:]
    im = p[:N1, CP:] + p[N1:, :CP]
    return re, im


def _ld(z_ref, rows):
    return jnp.concatenate([z_ref[c, rows, :] for c in range(4)], axis=1)


def _st(z_ref, rows, re, im):
    z_ref[0, rows, :] = re[:, :128]
    z_ref[1, rows, :] = re[:, 128:]
    z_ref[2, rows, :] = im[:, :128]
    z_ref[3, rows, :] = im[:, 128:]


NXC = S // TA


def _kernel(x_hbm, wr_hbm, wi_hbm, wg_hbm, wu_hbm, wd_hbm,
            cd_hbm, id_hbm, f1_ref, f1i_ref, gs_hbm, hs_hbm,
            o_ref,
            x_ref, wr_ref, wi_ref, wg_ref, wu_ref, wd_ref, cd_ref, id_ref,
            gs_ref, hs_ref, z_ref, wfr_ref, wfi_ref, xsem, sem):
    i = pl.program_id(0)

    def x_copy(t):
        return pltpu.make_async_copy(
            x_hbm.at[:, pl.ds(t * TA, TA)], x_ref.at[:, pl.ds(t * TA, TA)],
            xsem.at[t])

    big = [(cd_hbm, cd_ref), (wr_hbm, wr_ref), (wi_hbm, wi_ref),
           (gs_hbm, gs_ref), (hs_hbm, hs_ref), (id_hbm, id_ref),
           (wg_hbm, wg_ref), (wu_hbm, wu_ref), (wd_hbm, wd_ref)]

    def big_copy(k):
        return pltpu.make_async_copy(big[k][0], big[k][1], sem.at[k])

    @pl.when(i == 0)
    def _phase_a():
        x_copy(0).start()
        big_copy(0).start()

        big_copy(0).wait()
        x_copy(0).wait()
        for t in range(1, NXC):
            x_copy(t).start()
        for t in range(NXC):
            if t > 0:
                x_copy(t).wait()
            if t == NXC - 2:
                for k in range(1, 5):
                    big_copy(k).start()
            xf = x_ref[:, t * TA:(t + 1) * TA].astype(jnp.float32)
            zt = _ln_t(xf).astype(jnp.bfloat16)
            zz = jax.lax.dot_general(
                zt, cd_ref[...], (((0,), (0,)), ((), ())),
                preferred_element_type=jnp.float32)
            _st(z_ref, pl.ds(t * TA, TA), zz[:, :CP], zz[:, CP:])

        def body_s1(n2, c):
            zs = _ld(z_ref, pl.ds(n2, N1, stride=N2)).astype(jnp.bfloat16)
            p = jnp.dot(f1_ref[...], zs, preferred_element_type=jnp.float32)
            re, im = _cmul_split(p)
            _st(z_ref, pl.ds(n2, N1, stride=N2), re, im)
            return c
        jax.lax.fori_loop(0, N2, body_s1, 0, unroll=16)

        for k in range(5, len(big)):
            big_copy(k).start()

        big_copy(1).wait()
        big_copy(2).wait()
        wfr_ref[...] = jnp.zeros_like(wfr_ref)
        wfi_ref[...] = jnp.zeros_like(wfi_ref)
        for k2 in range(N2):
            wfr_ref[k2, :, 0:DF] = wr_ref[:, k2 * N1:(k2 + 1) * N1].astype(jnp.float32).T
            wfi_ref[k2, :, 0:DF] = wi_ref[:, k2 * N1:(k2 + 1) * N1].astype(jnp.float32).T

        big_copy(3).wait()
        big_copy(4).wait()

        def body_s2(g, c):
            r0 = pl.multiple_of(g * N1, N1)
            a = _ld(z_ref, pl.ds(r0, N1)).astype(jnp.bfloat16)
            p = jnp.dot(gs_ref[g], a, preferred_element_type=jnp.float32)
            xr, xi = _cmul_split(p)
            w0 = pl.multiple_of(g * 8, 8)
            wr = wfr_ref[:, pl.ds(w0, 8), :].reshape(N1, CP)
            wi = wfi_ref[:, pl.ds(w0, 8), :].reshape(N1, CP)
            yr = xr * wr - xi * wi
            yi = xr * wi + xi * wr
            y = jnp.concatenate([yr, yi], axis=1).astype(jnp.bfloat16)
            q = jnp.dot(hs_ref[g], y, preferred_element_type=jnp.float32)
            br, bi = _cmul_split(q)
            _st(z_ref, pl.ds(r0, N1), br, bi)
            return c
        jax.lax.fori_loop(0, NG, body_s2, 0, unroll=16)

        def body_s3(n2, c):
            zs = _ld(z_ref, pl.ds(n2, N1, stride=N2)).astype(jnp.bfloat16)
            p = jnp.dot(f1i_ref[...], zs, preferred_element_type=jnp.float32)
            re, im = _cmul_split(p)
            _st(z_ref, pl.ds(n2, N1, stride=N2), re, im)
            return c
        jax.lax.fori_loop(0, N2, body_s3, 0, unroll=16)

        for k in range(5, len(big)):
            big_copy(k).wait()

    r0 = pl.multiple_of(i * TM, TM)
    yb = _ld(z_ref, pl.ds(r0, TM)).astype(jnp.bfloat16)
    yt = jax.lax.dot_general(id_ref[...], yb, (((1,), (1,)), ((), ())),
                             preferred_element_type=jnp.float32)
    ht = x_ref[:, pl.ds(r0, TM)] + yt.astype(jnp.bfloat16)
    ln2 = _ln_t(ht.astype(jnp.float32)).T.astype(jnp.bfloat16)
    g = jnp.dot(ln2, wg_ref[...], preferred_element_type=jnp.float32).astype(jnp.bfloat16)
    u = jnp.dot(ln2, wu_ref[...], preferred_element_type=jnp.float32).astype(jnp.bfloat16)
    hh = g * u
    dn = jax.lax.dot_general(wd_ref[...], hh, (((1,), (1,)), ((), ())),
                             preferred_element_type=jnp.float32)
    o_ref[...] = ht + dn.astype(jnp.bfloat16)


@jax.jit
def pallas_sequential_preLN__spectral_gfnet__glu_gated_bilinear__prompt_kernel(
    A_x: jax.Array,
    A_w_r: jax.Array,
    A_w_i: jax.Array,
    B_x: jax.Array,
    B_w_gate: jax.Array,
    B_w_up: jax.Array,
    B_w_down: jax.Array,
):
    del B_x
    xt = A_x.reshape(S, D).T
    wrt = A_w_r.T
    wit = A_w_i.T
    wdt = B_w_down.T
    cd, idt, f1, f1i, gs, hs = (jnp.asarray(c) for c in _consts())

    full = lambda shape: pl.BlockSpec(shape, lambda i: (0,) * len(shape))
    anyspec = pl.BlockSpec(memory_space=pl.ANY)
    out = pl.pallas_call(
        _kernel,
        grid=(S // TM,),
        in_specs=[
            anyspec, anyspec, anyspec, anyspec, anyspec, anyspec,
            anyspec, anyspec, full(f1.shape), full(f1i.shape),
            anyspec, anyspec,
        ],
        out_specs=pl.BlockSpec((D, TM), lambda i: (0, i)),
        out_shape=jax.ShapeDtypeStruct((D, S), jnp.bfloat16),
        scratch_shapes=[
            pltpu.VMEM((D, S), jnp.bfloat16),
            pltpu.VMEM((DF, S), jnp.bfloat16),
            pltpu.VMEM((DF, S), jnp.bfloat16),
            pltpu.VMEM((D, FF), jnp.bfloat16),
            pltpu.VMEM((D, FF), jnp.bfloat16),
            pltpu.VMEM((D, FF), jnp.bfloat16),
            pltpu.VMEM(cd.shape, jnp.bfloat16),
            pltpu.VMEM(idt.shape, jnp.bfloat16),
            pltpu.VMEM(gs.shape, jnp.bfloat16),
            pltpu.VMEM(hs.shape, jnp.bfloat16),
            pltpu.VMEM((4, S, 128), jnp.float32),
            pltpu.VMEM((N2, N1, CP), jnp.float32),
            pltpu.VMEM((N2, N1, CP), jnp.float32),
            pltpu.SemaphoreType.DMA((NXC,)),
            pltpu.SemaphoreType.DMA((9,)),
        ],
        compiler_params=pltpu.CompilerParams(
            dimension_semantics=("arbitrary",),
            vmem_limit_bytes=100 * 1024 * 1024,
        ),
    )(xt, wrt, wit, B_w_gate, B_w_up, wdt, cd, idt, f1, f1i, gs, hs)
    return out.T.reshape(1, S, D)
```
